```python
import jax
import jax.numpy as jnp

def _softmax(x, axis=-1):
    return jax.nn.softmax(x, axis=axis)
def _gelu(x):
    return jax.nn.gelu(x, approximate=True)
def _silu(x):
    return jax.nn.silu(x)
def _sigmoid(x):
    return jax.nn.sigmoid(x)
def _layernorm(x, axis=-1, eps=1e-5):
    m = jnp.mean(x, axis=axis, keepdims=True)
    v = jnp.var(x, axis=axis, keepdims=True)
    return (x - m) / jnp.sqrt(v + eps)
def _scatter_add(tgt, idx, src, axis=0):
    return tgt.at[idx].add(src)
def _segment_sum(src, seg, n):
    return jax.ops.segment_sum(src, seg, n)
class _Rng:
    def __init__(self, key):
        self._k = key
    def _next(self):
        self._k, sub = jax.random.split(self._k)
        return sub
    def normal(self, shape):
        return jax.random.normal(self._next(), shape, dtype=jnp.bfloat16)
    def randint(self, lo, hi, shape):
        return jax.random.randint(self._next(), shape, lo, hi, dtype=jnp.int32)
    def uniform(self, shape, lo=0.0, hi=1.0):
        return jax.random.uniform(self._next(), shape, jnp.bfloat16, lo, hi)
    def permutation(self, n):
        return jax.random.permutation(self._next(), n)


kernel_name = 'standalone__modern_conv_block_replknet__vision'

def setup_inputs():
    _rng = _Rng(jax.random.key(int.from_bytes(__import__("os").urandom(4), "little")))
    _w = (lambda a: (lambda t: t.astype(jnp.bfloat16) if jnp.issubdtype(t.dtype, jnp.floating) else t)(jnp.asarray(a)))
    H = W = 512
    C = 96
    K = 3
    return {
        "x": _w((lambda *s: _rng.normal(s) * 0.05)(1, H, W, C)),
        "dw_large": _w((lambda *s: _rng.normal(s) * 0.05)(K, K, C) * (1.0 / K)),
        "dw_small": _w((lambda *s: _rng.normal(s) * 0.05)(5, 5, C) * 0.2),
        "w1": _w((lambda *s: _rng.normal(s) * 0.05)(C, 4 * C) * (C ** -0.5)),
        "w2": _w((lambda *s: _rng.normal(s) * 0.05)(4 * C, C) * ((4 * C) ** -0.5)),
    }

def reference(x, dw_large, dw_small, w1, w2):
    B, H, W, C = x.shape
    Kl = dw_large.shape[0]
    pl = (Kl - 1) // 2
    xpl = jnp.pad(x, ((0,0),(pl,pl),(pl,pl),(0,0)))
    out = jnp.zeros_like(x)
    for i in range(Kl):
        for j in range(Kl):
            out = out + xpl[:, i:i+H, j:j+W, :] * dw_large[i, j][None, None, None, :]
    Ks = dw_small.shape[0]
    ps = (Ks - 1) // 2
    xps = jnp.pad(x, ((0,0),(ps,ps),(ps,ps),(0,0)))
    for i in range(Ks):
        for j in range(Ks):
            out = out + xps[:, i:i+H, j:j+W, :] * dw_small[i, j][None, None, None, :]
    h = _layernorm(out, axis=-1)
    h = _gelu(jnp.einsum('bhwc,ce->bhwe', h, w1))
    h = jnp.einsum('bhwe,ec->bhwc', h, w2)
    return x + h
```

```python
import functools
import jax
import jax.numpy as jnp
import jax.experimental.pallas as pl
import jax.experimental.pallas.tpu as pltpu

TH = 64
CB = 8
UN = 4


def _body(xt_ref, x_ref, xb_ref, kl_ref, ks_ref, w1_ref, w2_ref, o_ref, xs_ref, k_ref, *, H, W, C):
    i = pl.program_id(0)
    f32 = jnp.float32

    @pl.when(i == 0)
    def _():
        ks = ks_ref[...].astype(f32).T
        kl = kl_ref[...].astype(f32).T
        for a in range(5):
            for b in range(5):
                k = ks[:, a * 5 + b:a * 5 + b + 1]
                if 1 <= a <= 3 and 1 <= b <= 3:
                    t = (a - 1) * 3 + b - 1
                    k = k + kl[:, t:t + 1]
                k_ref[a * 5 + b] = jnp.broadcast_to(k, (C, 128))

    xs_ref[0:2] = jnp.where(i > 0, xt_ref[...].astype(f32), 0.0)
    xs_ref[TH + 2:TH + 4] = jnp.where(i < H // TH - 1, xb_ref[...].astype(f32), 0.0)

    def cp(r, c):
        xs_ref[r + 2] = x_ref[r].astype(f32)
        return c
    jax.lax.fori_loop(0, TH, cp, 0)

    w1t = w1_ref[...].astype(f32).T.astype(jnp.bfloat16)
    w2t = w2_ref[...] * jnp.bfloat16(0.5)
    lane = jax.lax.broadcasted_iota(jnp.int32, (CB, 128), 1)
    NT = W // 128

    def conv(r):
        outs = []
        for c0 in range(0, C, CB):
            acc = [None] * NT
            for b in range(5):
                s = 2 - b
                p = []
                for t in range(NT):
                    q = None
                    for a in range(5):
                        v = xs_ref[r + a, c0:c0 + CB, t * 128:(t + 1) * 128] * k_ref[a * 5 + b, c0:c0 + CB, :]
                        q = v if q is None else q + v
                    p.append(pltpu.roll(q, s % 128, 1) if s else q)
                for t in range(NT):
                    if s > 0:
                        q = jnp.where(lane >= s, p[t], p[t - 1] if t > 0 else 0.0)
                    elif s < 0:
                        q = jnp.where(lane < 128 + s, p[t], p[t + 1] if t < NT - 1 else 0.0)
                    else:
                        q = p[t]
                    acc[t] = q if acc[t] is None else acc[t] + q
            outs.append(jnp.concatenate(acc, axis=1))
        acc = jnp.concatenate(outs, axis=0)
        m = jnp.mean(acc, axis=0, keepdims=True)
        d = acc - m
        var = jnp.mean(d * d, axis=0, keepdims=True)
        return (d * jax.lax.rsqrt(var + 1e-5)).astype(jnp.bfloat16)

    def mlp(r, h):
        u = jnp.dot(w1t, h, preferred_element_type=f32)
        z = u * (0.7978845608028654 + (0.7978845608028654 * 0.044715) * (u * u))
        g = (u * jnp.tanh(z) + u).astype(jnp.bfloat16)
        y = jnp.dot(w2t, g, preferred_element_type=f32)
        o_ref[r] = (xs_ref[r + 2] + y).astype(o_ref.dtype)

    def row(j, h):
        for q in range(UN):
            r = j * UN + q
            hn = conv(jnp.minimum(r + 1, TH - 1))
            mlp(r, h)
            h = hn
        return h
    jax.lax.fori_loop(0, TH // UN, row, conv(0))


@jax.jit
def pallas_standalone__modern_conv_block_replknet__vision_kernel(x, dw_large, dw_small, w1, w2):
    B, H, W, C = x.shape
    xt = x.reshape(H, W, C).transpose(0, 2, 1)
    n = H // TH
    hb = TH // 2
    full = lambda s: pl.BlockSpec(s, lambda i: (0,) * len(s))
    out = pl.pallas_call(
        functools.partial(_body, H=H, W=W, C=C),
        grid=(n,),
        in_specs=[
            pl.BlockSpec((2, C, W), lambda i: (jnp.maximum(i * hb - 1, 0), 0, 0)),
            pl.BlockSpec((TH, C, W), lambda i: (i, 0, 0)),
            pl.BlockSpec((2, C, W), lambda i: (jnp.minimum((i + 1) * hb, H // 2 - 1), 0, 0)),
            full((9, C)), full((25, C)), full(w1.shape), full((C, 4 * C)),
        ],
        out_specs=pl.BlockSpec((TH, C, W), lambda i: (i, 0, 0)),
        out_shape=jax.ShapeDtypeStruct((H, C, W), x.dtype),
        scratch_shapes=[pltpu.VMEM((TH + 4, C, W), jnp.float32), pltpu.VMEM((25, C, 128), jnp.float32)],
        compiler_params=pltpu.CompilerParams(dimension_semantics=("arbitrary",), vmem_limit_bytes=100 << 20),
    )(xt, xt, xt, dw_large.reshape(9, C), dw_small.reshape(25, C), w1, w2.T)
    return out.transpose(0, 2, 1).reshape(B, H, W, C)
```
